```python
import os as _os
_os.environ.setdefault('JAX_PLATFORMS', 'cpu')
import jax
import jax.numpy as jnp

def _softmax(x, axis=-1):
    return jax.nn.softmax(x, axis=axis)

def _gelu(x):
    return jax.nn.gelu(x, approximate=True)

def _silu(x):
    return jax.nn.silu(x)

def _sigmoid(x):
    return jax.nn.sigmoid(x)

def _layernorm(x, axis=-1, eps=1e-05):
    m = jnp.mean(x, axis=axis, keepdims=True)
    v = jnp.var(x, axis=axis, keepdims=True)
    return (x - m) / jnp.sqrt(v + eps)

def _scatter_add(tgt, idx, src, axis=0):
    return tgt.at[idx].add(src)

def _segment_sum(src, seg, n):
    return jax.ops.segment_sum(src, seg, n)

class _Rng:

    def __init__(self, key):
        self._k = key

    def _next(self):
        self._k, sub = jax.random.split(self._k)
        return sub

    def normal(self, shape):
        return jax.random.normal(self._next(), shape, dtype=jnp.bfloat16)

    def randint(self, lo, hi, shape):
        return jax.random.randint(self._next(), shape, lo, hi, dtype=jnp.int32)

    def uniform(self, shape, lo=0.0, hi=1.0):
        return jax.random.uniform(self._next(), shape, jnp.bfloat16, lo, hi)

    def permutation(self, n):
        return jax.random.permutation(self._next(), n)
kernel_name = 'adaLN_cond__mha_block_cached__geglu_ffn__prompt'

def setup_inputs():
    _rng = _Rng(jax.random.key(int.from_bytes(__import__("os").urandom(4), "little")))
    _w = lambda a: (lambda t: t.astype(jnp.bfloat16) if jnp.issubdtype(t.dtype, jnp.floating) else t)(jnp.asarray(a))

    def _A_setup():
        B, Sq, D = (1, 2048, 512)
        H, Sk, Dh = (32, 2048, 128)
        return {'x': _w((lambda *s: _rng.normal(s) * 0.05)(B, Sq, D)), 'k_cache': _w((lambda *s: _rng.normal(s) * 3.2)(B, H, Sk, Dh)), 'v_cache': _w((lambda *s: _rng.normal(s) * 0.4)(B, H, Sk, Dh)), 'wq': _w((lambda *s: _rng.normal(s) * 1.6)(D, H * Dh) * D ** (-0.5)), 'wo': _w((lambda *s: _rng.normal(s) * 0.4)(H * Dh, D) * (H * Dh) ** (-0.5))}
    _A_in = _A_setup()

    def _B_setup():
        B, S, D, F = (1, 2048, 512, 1792)
        return {'x': _w((lambda *s: _rng.normal(s) * 0.05)(B, S, D)), 'w_gate': _w((lambda *s: _rng.normal(s) * 0.05)(D, F)), 'w_up': _w((lambda *s: _rng.normal(s) * 0.05)(D, F)), 'w_down': _w((lambda *s: _rng.normal(s) * 0.05)(F, D))}
    _B_in = _B_setup()
    return {'A_x': _A_in['x'], 'A_k_cache': _A_in['k_cache'], 'A_v_cache': _A_in['v_cache'], 'A_wq': _A_in['wq'], 'A_wo': _A_in['wo'], 'B_x': _B_in['x'], 'B_w_gate': _B_in['w_gate'], 'B_w_up': _B_in['w_up'], 'B_w_down': _B_in['w_down'], 'c': _w((lambda *s: _rng.normal(s) * 0.05)(1, 512) * 8.0), 'w_mod': _w((lambda *s: _rng.normal(s) * 0.05)(512, 6 * 512) * 512 ** (-0.5) * 8.0)}

def reference(A_x, A_k_cache, A_v_cache, A_wq, A_wo, B_x, B_w_gate, B_w_up, B_w_down, c, w_mod):

    def _A_ref(x, k_cache, v_cache, wq, wo):
        B, Sq, D = x.shape
        H, Dh = (32, 128)
        q = (lambda x, *d: x.transpose(*d))((x @ wq).reshape(B, Sq, H, Dh), 0, 2, 1, 3)
        scores = jnp.einsum('bhqd,bhkd->bhqk', q, k_cache) * Dh ** (-0.5)
        p = _softmax(scores, axis=-1)
        o = jnp.einsum('bhqk,bhkd->bhqd', p, v_cache)
        return (lambda x, *d: x.transpose(*d))(o, 0, 2, 1, 3).reshape(B, Sq, H * Dh) @ wo

    def _B_ref(x, w_gate, w_up, w_down):
        return _gelu(x @ w_gate) * (x @ w_up) @ w_down
    x = A_x
    mod = (_silu(c) @ w_mod).reshape(c.shape[0], 6, 1, -1)
    sa, ca, ga, sb, cb, gb = (mod[:, 0].copy(), mod[:, 1].copy(), mod[:, 2].copy(), mod[:, 3].copy(), mod[:, 4].copy(), mod[:, 5].copy())
    h = _layernorm(x, axis=-1) * (1 + ca) + sa
    x = x + ga * _A_ref(h, A_k_cache, A_v_cache, A_wq, A_wo)
    h = _layernorm(x, axis=-1) * (1 + cb) + sb
    x = x + gb * _B_ref(h, B_w_gate, B_w_up, B_w_down)
    return x
```

```python
import functools
import numpy as np
import jax
import jax.numpy as jnp
import jax.experimental.pallas as pl
import jax.experimental.pallas.tpu as pltpu

S, D, H, SK, DH, F = 2048, 512, 32, 2048, 128, 1792
BQ = 256
RB = 256
G = 512
FLAGS = None
DEP = 1
DEP2 = 2
RCP = 1
PACE = 1
LAG = 1
XCH = 512
FINAL = 'pipe'
NOBC = 1
HUNROLL = 1
NPRE = 16
HLATE = 8

LOG2E = 1.4426950408889634
QSCALE = float(DH ** -0.5 * LOG2E)
NG = SK // G
NB = S // BQ
NX = S // XCH
NR = S // RB


def _ln(x):
    m = jnp.mean(x, axis=-1, keepdims=True)
    xc = x - m
    v = jnp.mean(xc * xc, axis=-1, keepdims=True)
    return xc * jax.lax.rsqrt(v + 1e-5)


def _kernel(x_hbm, k_hbm, v_hbm, wq_hbm, wo_hbm, wg_hbm, wu_hbm, wd_hbm, c_hbm, wmod_hbm,
            out_hbm,
            x_s, kvq_s, wo_s, wg_s, wu_s, wd_s, c_s, wmod_s, x1_s, h2_s, h_s, o_s, out_s,
            sem_c, sem_x, sem_kvq, sem_w, sem_out):

    def c_copy():
        return pltpu.make_async_copy(c_hbm, c_s, sem_c.at[0])

    def moda_copy():
        return pltpu.make_async_copy(wmod_hbm.at[:, 0:2 * D], wmod_s.at[:, 0:2 * D], sem_c.at[1])

    def modb_copy():
        return pltpu.make_async_copy(wmod_hbm.at[:, 2 * D:], wmod_s.at[:, 2 * D:], sem_w.at[0])

    def x_copy(i):
        r = i * XCH if isinstance(i, int) else pl.multiple_of(i * XCH, XCH)
        return pltpu.make_async_copy(x_hbm.at[pl.ds(r, XCH), :], x_s.at[pl.ds(r, XCH), :], sem_x.at[i])

    def kvq_copies(h):
        c0 = h * DH if isinstance(h, int) else pl.multiple_of(h * DH, DH)
        return (pltpu.make_async_copy(wq_hbm.at[:, pl.ds(c0, DH)], kvq_s.at[h, pl.ds(0, D)], sem_kvq.at[h]),
                pltpu.make_async_copy(k_hbm.at[h], kvq_s.at[h, pl.ds(D, SK)], sem_kvq.at[h]),
                pltpu.make_async_copy(v_hbm.at[h], kvq_s.at[h, pl.ds(D + SK, SK)], sem_kvq.at[h]))

    def kvq_wait(h):
        pltpu.make_async_copy(kvq_s.at[h], kvq_s.at[h], sem_kvq.at[h]).wait()

    def w_copies():
        return (modb_copy(),
                pltpu.make_async_copy(wo_hbm, wo_s, sem_w.at[1]),
                pltpu.make_async_copy(wg_hbm, wg_s, sem_w.at[2]),
                pltpu.make_async_copy(wu_hbm, wu_s, sem_w.at[3]),
                pltpu.make_async_copy(wd_hbm, wd_s, sem_w.at[4]))

    def out_copy(r0):
        return pltpu.make_async_copy(out_s.at[pl.ds(r0, RB), :], out_hbm.at[pl.ds(r0, RB), :], sem_out)

    with jax.named_scope("prologue"):
        c_copy().start()
        moda_copy().start()

        def start_x(i, carry):
            x_copy(i).start()
            return carry
        jax.lax.fori_loop(0, NX, start_x, 0)

        def start_kvq(h, carry):
            for cp in kvq_copies(h):
                cp.start()
            return carry
        jax.lax.fori_loop(0, NPRE, start_kvq, 0)
        c_copy().wait()
        moda_copy().wait()
        c = c_s[...].astype(jnp.float32)
        sc = (c * jax.nn.sigmoid(c)).astype(jnp.bfloat16)
        sc8 = jnp.broadcast_to(sc, (16, D))
        moda = jnp.dot(sc8, wmod_s[:, 0:2 * D], preferred_element_type=jnp.float32)[0:8]
        sa = moda[0:1, 0:D]
        ca1 = 1.0 + moda[0:1, D:2 * D]
        for r in range(NX):
            x_copy(r).wait()
            x = x_s[r * XCH:(r + 1) * XCH, :].astype(jnp.float32)
            h_s[r * XCH:(r + 1) * XCH, :] = (_ln(x) * ca1 + sa).astype(jnp.bfloat16)

    def head_body(h, carry):
        kvq_wait(h)

        @pl.when(h == HLATE)
        def _():
            for hh in range(NPRE, H):
                for cp in kvq_copies(hh):
                    cp.start()
            for cp in w_copies():
                cp.start()

        never = h > 1000
        wq_ref = kvq_s.at[h, pl.ds(0, D)]
        k_ref = kvq_s.at[h, pl.ds(D, SK)]
        v_ref = kvq_s.at[h, pl.ds(D + SK, SK)]

        def qk(q, g):
            return jax.lax.dot_general(q, k_ref[g * G:(g + 1) * G, :], (((1,), (1,)), ((), ())),
                                       preferred_element_type=jnp.float32)

        def tiles(s):
            return [s[:, t * 128:(t + 1) * 128] for t in range(s.shape[1] // 128)]

        def tree(f, xs):
            while len(xs) > 1:
                xs = [f(xs[i], xs[i + 1]) if i + 1 < len(xs) else xs[i] for i in range(0, len(xs), 2)]
            return xs[0]

        def pv(s, mfull, g, l, pace):
            ts = tiles(s)
            if pace is not None:
                mfull = jnp.where(never, pace, mfull)
            ts = [jnp.exp2(t - mfull) for t in ts]
            dl = tree(jnp.add, ts)
            l = dl if l is None else l + dl
            if DEP:
                ts[-1] = jnp.where(never, l, ts[-1])
            pb = jnp.concatenate(ts, axis=1).astype(jnp.bfloat16)
            return l, jnp.dot(pb, v_ref[g * G:(g + 1) * G, :], preferred_element_type=jnp.float32)

        def rowmax(ss):
            mm = tree(jnp.maximum, [t for s in ss for t in tiles(s)])
            return jnp.broadcast_to(jnp.max(mm, axis=-1, keepdims=True), (BQ, 128))

        def finish(acc, l):
            lsum = jnp.sum(l, axis=-1, keepdims=True)
            if RCP:
                r = pl.reciprocal(lsum, approx=True)
                r = r * (2.0 - lsum * r)
                return acc * r
            return acc / lsum

        def run_blocks(base, nblk):
            def r0(b):
                return base + b * BQ
            stages = [('Q', 0), ('Q', 1)] + [('K', 0, g) for g in range(NG)]
            for b in range(nblk):
                if b + 1 < nblk:
                    stages += [('K', b + 1, g) for g in range(NG)]
                if b + 2 < nblk:
                    stages += [('Q', b + 2)]
                stages += [('P', b, g) for g in range(NG)]
            q = {}; ss = {}; m = {}; l = {}; acc = {}; onorm = {}
            hist = []
            for st in stages:
                if st[0] == 'Q':
                    b = st[1]
                    hq = h_s[pl.ds(r0(b), BQ), :]
                    qf = jnp.dot(hq, wq_ref[...], preferred_element_type=jnp.float32)
                    q[b] = (qf * QSCALE).astype(jnp.bfloat16)
                    hist.append(qf)
                elif st[0] == 'K':
                    _, b, g = st
                    s = qk(q[b], g)
                    ss[b, g] = s
                    hist.append(s[:, 0:128])
                    if g == NG - 1:
                        m[b] = rowmax([ss[b, gg] for gg in range(NG)])
                else:
                    _, b, g = st
                    pace = hist[-LAG] if PACE else None
                    if DEP2 and g == DEP2 and b > 0:
                        pace = onorm[b - 1] if pace is None else jnp.where(never, onorm[b - 1], pace)
                    l[b], do = pv(ss[b, g], m[b], g, l.get(b), pace)
                    acc[b] = do if g == 0 else acc[b] + do
                    hist.append(do)
                    if g == NG - 1:
                        onorm[b] = finish(acc[b], l[b])
                        o_s[h, pl.ds(r0(b), BQ), :] = onorm[b].astype(jnp.bfloat16)

        run_blocks(0, NB)
        return carry

    with jax.named_scope("attn"):
        jax.lax.fori_loop(0, H, head_body, 0, unroll=HUNROLL)

    with jax.named_scope("final"):
        for cp in w_copies():
            cp.wait()
        modb = jnp.dot(sc8, wmod_s[:, 2 * D:], preferred_element_type=jnp.float32)[0:8]
        ga = modb[0:1, 0:D]
        sb = modb[0:1, D:2 * D]
        cb1 = 1.0 + modb[0:1, 2 * D:3 * D]
        gb = modb[0:1, 3 * D:4 * D]

        def op_part(r0):
            o = jnp.concatenate([o_s[hh, pl.ds(r0, RB), :] for hh in range(H)], axis=1)
            attn = jnp.dot(o, wo_s[...], preferred_element_type=jnp.float32)
            x1 = x_s[pl.ds(r0, RB), :].astype(jnp.float32) + ga * attn
            h2 = (_ln(x1) * cb1 + sb).astype(jnp.bfloat16)
            return x1, h2

        def ffn_part(r0, x1, h2):
            g = jnp.dot(h2, wg_s[...], preferred_element_type=jnp.float32)
            u = jnp.dot(h2, wu_s[...], preferred_element_type=jnp.float32)
            a = (jax.nn.gelu(g, approximate=True) * u).astype(jnp.bfloat16)
            y = jnp.dot(a, wd_s[...], preferred_element_type=jnp.float32)
            out_s[pl.ds(r0, RB), :] = (x1 + gb * y).astype(out_s.dtype)
            out_copy(r0).start()

        if FINAL == 'loop':
            def body(i, carry):
                r0 = pl.multiple_of(i * RB, RB)
                x1, h2 = op_part(r0)
                ffn_part(r0, x1, h2)
                return carry
            jax.lax.fori_loop(0, NR, body, 0)
        elif FINAL == 'unroll':
            nxt = op_part(0)
            for i in range(NR):
                cur = nxt
                if i + 1 < NR:
                    nxt = op_part((i + 1) * RB)
                ffn_part(i * RB, *cur)
        elif FINAL == 'pipe':
            x1, h2 = op_part(0)
            x1_s[...] = x1
            h2_s[...] = h2

            def body(i, carry):
                r0 = pl.multiple_of(i * RB, RB)
                x1 = x1_s[...]
                h2 = h2_s[...]
                x1n, h2n = op_part(pl.multiple_of(r0 + RB, RB))
                ffn_part(r0, x1, h2)
                x1_s[...] = x1n
                h2_s[...] = h2n
                return carry
            jax.lax.fori_loop(0, NR - 1, body, 0)
            ffn_part((NR - 1) * RB, x1_s[...], h2_s[...])

        pltpu.make_async_copy(out_s, out_hbm, sem_out).wait()


@jax.jit
def pallas_adaLN_cond__mha_block_cached__geglu_ffn__prompt_kernel(A_x, A_k_cache, A_v_cache, A_wq, A_wo, B_x, B_w_gate, B_w_up, B_w_down, c, w_mod):
    x = A_x.reshape(S, D)
    k = A_k_cache.reshape(H, SK, DH)
    v = A_v_cache.reshape(H, SK, DH)
    anyspec = pl.BlockSpec(memory_space=pl.ANY)
    bf = jnp.bfloat16
    out = pl.pallas_call(
        _kernel,
        in_specs=[anyspec] * 10,
        out_specs=anyspec,
        out_shape=jax.ShapeDtypeStruct((S, D), bf),
        scratch_shapes=[
            pltpu.VMEM((S, D), bf),
            pltpu.VMEM((H, D + 2 * SK, DH), bf),
            pltpu.VMEM((H * DH, D), bf),
            pltpu.VMEM((D, F), bf),
            pltpu.VMEM((D, F), bf),
            pltpu.VMEM((F, D), bf),
            pltpu.VMEM((1, D), bf),
            pltpu.VMEM((D, 6 * D), bf),
            pltpu.VMEM((RB, D), jnp.float32),
            pltpu.VMEM((RB, D), bf),
            pltpu.VMEM((S, D), bf),
            pltpu.VMEM((H, S, DH), bf),
            pltpu.VMEM((S, D), bf),
            pltpu.SemaphoreType.DMA((2,)),
            pltpu.SemaphoreType.DMA((NX,)),
            pltpu.SemaphoreType.DMA((H,)),
            pltpu.SemaphoreType.DMA((5,)),
            pltpu.SemaphoreType.DMA(()),
        ],
        compiler_params=pltpu.CompilerParams(
            vmem_limit_bytes=100 * 1024 * 1024, flags=FLAGS,
            disable_bounds_checks=bool(NOBC),
        ),
    )(x, k, v, A_wq, A_wo, B_w_gate, B_w_up, B_w_down, c, w_mod)
    return out.reshape(1, S, D)
```

```python
import functools
import numpy as np
import jax
import jax.numpy as jnp
import jax.experimental.pallas as pl
import jax.experimental.pallas.tpu as pltpu

S, D, H, SK, DH, F = 2048, 512, 32, 2048, 128, 1792
BQ = 256
RB = 256
G = 512
FLAGS = None
DEP = 1
LAG = 1
XCH = 256
NOBC = 1
NOSC = 1
NPRE = 12
HL1 = 4
N1 = 24
HL2 = 12
FUNROLL = 2
OPOS = 0
PACE = 1
PEEL = 1
XW = 0
BC = 1
TAIL = 0
X1 = 0
OSPLIT = 2

LOG2E = 1.4426950408889634
QSCALE = float(DH ** -0.5 * LOG2E)
NG = SK // G
NB = S // BQ
NX = S // XCH
NR = S // RB


def _ln(x):
    m = jnp.mean(x, axis=-1, keepdims=True)
    xc = x - m
    v = jnp.mean(xc * xc, axis=-1, keepdims=True)
    return xc * jax.lax.rsqrt(v + 1e-5)


def _tiles(s):
    return [s[:, t * 128:(t + 1) * 128] for t in range(s.shape[1] // 128)]


def _tree(f, xs):
    while len(xs) > 1:
        xs = [f(xs[i], xs[i + 1]) if i + 1 < len(xs) else xs[i] for i in range(0, len(xs), 2)]
    return xs[0]


def _kernel(x_hbm, k_hbm, v_hbm, wq_hbm, wo_hbm, wg_hbm, wu_hbm, wd_hbm, c_hbm, wmod_hbm,
            out_hbm,
            x_s, kvq_s, wo_s, wg_s, wu_s, wd_s, c_s, wmod_s, h_s, acc_s, x1_s, olast_s, out_s,
            sem_c, sem_x, sem_kvq, sem_h0, sem_w, sem_out):

    def c_copy():
        return pltpu.make_async_copy(c_hbm, c_s, sem_c.at[0])

    def moda_copy():
        return pltpu.make_async_copy(wmod_hbm.at[:, 0:2 * D], wmod_s.at[:, 0:2 * D], sem_c.at[1])

    def x_copy(i):
        r = i * XCH if isinstance(i, int) else pl.multiple_of(i * XCH, XCH)
        return pltpu.make_async_copy(x_hbm.at[pl.ds(r, XCH), :], x_s.at[pl.ds(r, XCH), :], sem_x.at[i])

    def head_copies(h):
        c0 = h * DH if isinstance(h, int) else pl.multiple_of(h * DH, DH)
        return (pltpu.make_async_copy(wq_hbm.at[:, pl.ds(c0, DH)], kvq_s.at[h, pl.ds(0, D)], sem_kvq.at[h]),
                pltpu.make_async_copy(k_hbm.at[h], kvq_s.at[h, pl.ds(D, SK)], sem_kvq.at[h]),
                pltpu.make_async_copy(v_hbm.at[h], kvq_s.at[h, pl.ds(D + SK, SK)], sem_kvq.at[h]),
                pltpu.make_async_copy(wo_hbm.at[pl.ds(c0, DH), :], wo_s.at[h], sem_kvq.at[h]))

    def head0_copies():
        return (pltpu.make_async_copy(wq_hbm.at[:, pl.ds(0, DH)], kvq_s.at[0, pl.ds(0, D)], sem_h0.at[0]),
                pltpu.make_async_copy(k_hbm.at[0], kvq_s.at[0, pl.ds(D, SK)], sem_h0.at[1]),
                pltpu.make_async_copy(v_hbm.at[0], kvq_s.at[0, pl.ds(D + SK, SK)], sem_h0.at[2]),
                pltpu.make_async_copy(wo_hbm.at[pl.ds(0, DH), :], wo_s.at[0], sem_h0.at[3]))

    def w_copies():
        return (pltpu.make_async_copy(wmod_hbm.at[:, 2 * D:], wmod_s.at[:, 2 * D:], sem_w.at[0]),
                pltpu.make_async_copy(wg_hbm, wg_s, sem_w.at[1]),
                pltpu.make_async_copy(wu_hbm, wu_s, sem_w.at[2]),
                pltpu.make_async_copy(wd_hbm, wd_s, sem_w.at[3]))

    def out_copy(r0, n):
        r0 = pl.multiple_of(r0, n)
        return pltpu.make_async_copy(out_s.at[pl.ds(r0, n), :], out_hbm.at[pl.ds(r0, n), :], sem_out)

    with jax.named_scope("prologue"):
        if not PEEL:
            c_copy().start()
            moda_copy().start()

        if PEEL:
            hc0 = head0_copies()
            order = [c_copy(), moda_copy(), x_copy(0), x_copy(1), hc0[0], hc0[1], hc0[2], x_copy(2), x_copy(3), hc0[3]] + \
                    [x_copy(i) for i in range(4, NX)]

            def start_first(i, carry):
                for k, cp in enumerate(order):
                    pl.when(i == k)(cp.start)
                return carry
            jax.lax.fori_loop(0, len(order), start_first, 0)

            def start_head(h, carry):
                for cp in head_copies(h):
                    cp.start()
                return carry + 1
            cnt = jax.lax.fori_loop(1, NPRE, start_head, 0)
        else:
            def start_x(i, carry):
                x_copy(i).start()
                return carry
            jax.lax.fori_loop(0, NX, start_x, 0)

            def start_head(h, carry):
                for cp in head_copies(h):
                    cp.start()
                return carry + 1
            cnt = jax.lax.fori_loop(0, NPRE, start_head, 0)
        if PEEL:
            acc_s[(NB - 1) * BQ:, :] = jnp.zeros((BQ, D), jnp.float32)
        else:
            acc_s[...] = jnp.zeros(acc_s.shape, jnp.float32)
            olast_s[...] = jnp.zeros(olast_s.shape, jnp.bfloat16)
        c_copy().wait()
        moda_copy().wait()
        c = c_s[...].astype(jnp.float32)
        sc = (c * jax.nn.sigmoid(c)).astype(jnp.bfloat16)
        sc8 = jnp.broadcast_to(sc, (16, D))
        moda = jnp.dot(sc8, wmod_s[:, 0:2 * D], preferred_element_type=jnp.float32)[0:8]
        sa = moda[0:1, 0:D]
        ca1 = 1.0 + moda[0:1, D:2 * D]
        if not PEEL:
            for r in range(NX):
                x_copy(r).wait()
                x = x_s[r * XCH:(r + 1) * XCH, :].astype(jnp.float32)
                h_s[r * XCH:(r + 1) * XCH, :] = (_ln(x) * ca1 + sa).astype(jnp.bfloat16)

    def head_body(h, carry, first=False):
        if first:
            hc = head0_copies()
            waited = set()

            def need(name):
                if name in waited:
                    return
                waited.add(name)
                if name == 'wq': hc[0].wait()
                elif name == 'k': hc[1].wait()
                elif name == 'v': hc[2].wait()
                elif name == 'wo': hc[3].wait()
                else: x_copy(int(name[1:])).wait()
        else:
            for cp in head_copies(h):
                cp.wait()

            def need(name):
                pass

        if not first:
            _late(h)
        return head_main(h, carry, first, need)

    def _late(h):
        @pl.when(h == HL1)
        def _():
            for hh in range(NPRE, N1):
                for cp in head_copies(hh):
                    cp.start()

        @pl.when(h == HL2)
        def _():
            for hh in range(N1, H):
                for cp in head_copies(hh):
                    cp.start()
            for cp in w_copies():
                cp.start()

    def head_main(h, carry, first, need):
        never = (cnt > 1000) if first else (h > 1000)
        kvq32 = kvq_s.bitcast(jnp.uint32)

        def ld(r0, n):
            if BC:
                return pltpu.bitcast(kvq32[h, r0 // 2:(r0 + n) // 2, :], jnp.bfloat16)
            return kvq_s[h, r0:r0 + n, :]
        wo_ref = wo_s.at[h]
        wo_prev = wo_s.at[jnp.maximum(h - 1, 0)]

        def qk(q, g):
            return jax.lax.dot_general(q, ld(D + g * G, G), (((1,), (1,)), ((), ())),
                                       preferred_element_type=jnp.float32)

        def pv(s, mfull, g, l, pace):
            ts = _tiles(s)
            if pace is not None:
                mfull = jnp.where(never, pace, mfull)
            ts = [jnp.exp2(t - mfull) for t in ts]
            dl = _tree(jnp.add, ts)
            l = dl if l is None else l + dl
            if DEP:
                ts[-1] = jnp.where(never, l, ts[-1])
            pb = jnp.concatenate(ts, axis=1).astype(jnp.bfloat16)
            return l, jnp.dot(pb, ld(D + SK + g * G, G), preferred_element_type=jnp.float32)

        def rowmax(ss):
            mm = _tree(jnp.maximum, [t for s in ss for t in _tiles(s)])
            return jnp.broadcast_to(jnp.max(mm, axis=-1, keepdims=True), (BQ, 128))

        def finish(acc, l):
            lsum = jnp.sum(l, axis=-1, keepdims=True)
            r = pl.reciprocal(lsum, approx=True)
            r = r * (2.0 - lsum * r)
            return (acc * r).astype(jnp.bfloat16)

        def oproj(b, o, w_ref):
            y = jnp.dot(o, w_ref[...], preferred_element_type=jnp.float32)
            if first:
                acc_s[b * BQ:(b + 1) * BQ, :] = y
            else:
                acc_s[b * BQ:(b + 1) * BQ, :] += y
            return y

        def KK(b): return [('K', b, g) for g in range(NG)]
        def PP(b): return [('P', b, g) for g in range(NG)]
        if first:
            stages = [('W', 'x0', 'x1', 'wq'), ('Q', 0), ('Q', 1), ('W', 'k')] + KK(0) + KK(1)
            stages += [('W', 'v', 'x2', 'x3', 'wo')] + PP(0) + [('Q', 2)] + KK(2) + [('O', 0), ('Q', 3)] + PP(1) + KK(3)
            stages += [('W', 'x4', 'x5', 'x6', 'x7'), ('O', 1)] + PP(2) + [('Q', 4)] + KK(4) + [('O', 2), ('Q', 5)] + PP(3) + KK(5)
            stages += [('O', 3), ('Q', 6)] + PP(4) + KK(6) + [('O', 4), ('Q', 7)] + PP(5) + KK(7) + [('O', 5)] + PP(6) + [('O', 6)] + PP(7)
        else:
          stages = [('Q', 0), ('Q', 1)] + [('K', 0, g) for g in range(NG)]
          for b in range(NB):
            if b + 1 < NB:
                stages += [('K', b + 1, g) for g in range(NG)]
            if OPOS == 0:
                stages += [('O', b - 1)]
            if b + 2 < NB:
                stages += [('Q', b + 2)]
            if OPOS == 1:
                stages += [('O', b - 1)]
            stages += [('P', b, g) for g in range(NG)]
          if TAIL == 1:
            stages.remove(('O', NB - 2))
            stages.append(('O', NB - 2))
        q = {}; ss = {}; m = {}; l = {}; acc = {}; onorm = {}
        hist = []
        hq_pre = {}
        for st in stages:
            if st[0] == 'W':
                for name in st[1:]:
                    need(name)
                for name in st[1:]:
                    if name[0] == 'x':
                        b = int(name[1:])
                        xx = x_s[b * BQ:(b + 1) * BQ, :].astype(jnp.float32)
                        hq_pre[b] = (_ln(xx) * ca1 + sa).astype(jnp.bfloat16)
                        h_s[b * BQ:(b + 1) * BQ, :] = hq_pre[b]
            elif st[0] == 'Q':
                b = st[1]
                if first:
                    hq = hq_pre[b]
                elif False:
                    xx = x_s[b * BQ:(b + 1) * BQ, :].astype(jnp.float32)
                    hq = (_ln(xx) * ca1 + sa).astype(jnp.bfloat16)
                    h_s[b * BQ:(b + 1) * BQ, :] = hq
                else:
                    hq = h_s[b * BQ:(b + 1) * BQ, :]
                need('wq')
                qf = jnp.dot(hq, ld(0, D), preferred_element_type=jnp.float32)
                q[b] = (qf * QSCALE).astype(jnp.bfloat16)
                hist.append(qf)
            elif st[0] == 'K':
                _, b, g = st
                need('k')
                s = qk(q[b], g)
                ss[b, g] = s
                hist.append(s[:, 0:128])
                if g == NG - 1:
                    m[b] = rowmax([ss[b, gg] for gg in range(NG)])
            elif st[0] == 'O':
                b = st[1]
                if b < 0:
                    if first:
                        continue
                    y = oproj(NB - 1, olast_s[...], wo_prev)
                else:
                    need('wo')
                    y = oproj(b, onorm[b], wo_ref)
                hist.append(y[:, 0:128])
            else:
                _, b, g = st
                need('v')
                pace = hist[-LAG] if PACE else None
                l[b], do = pv(ss[b, g], m[b], g, l.get(b), pace)
                acc[b] = do if g == 0 else acc[b] + do
                hist.append(do)
                if g == NG - 1:
                    onorm[b] = finish(acc[b], l[b])
                    if b == NB - 1:
                        olast_s[...] = onorm[b]
        return carry

    if PEEL:
        with jax.named_scope("head0"):
            head_body(0, 0, first=True)
    with jax.named_scope("attn"):
        jax.lax.fori_loop(1 if PEEL else 0, H, head_body, 0)

    with jax.named_scope("final"):
        for cp in w_copies():
            cp.wait()
        acc_s[(NB - 1) * BQ:, :] += jnp.dot(olast_s[...], wo_s[H - 1], preferred_element_type=jnp.float32)
        modb = jnp.dot(sc8, wmod_s[:, 2 * D:], preferred_element_type=jnp.float32)[0:8]
        ga = modb[0:1, 0:D]
        sb = modb[0:1, D:2 * D]
        cb1 = 1.0 + modb[0:1, 2 * D:3 * D]
        gb = modb[0:1, 3 * D:4 * D]

        def ln_part(r0):
            x1 = x_s[pl.ds(r0, RB), :].astype(jnp.float32) + ga * acc_s[pl.ds(r0, RB), :]
            if X1:
                x1_s[pl.ds(r0, RB), :] = x1
            h_s[pl.ds(r0, RB), :] = (_ln(x1) * cb1 + sb).astype(jnp.bfloat16)

        def ffn_part(r0, h2):
            g = jnp.dot(h2, wg_s[...], preferred_element_type=jnp.float32)
            u = jnp.dot(h2, wu_s[...], preferred_element_type=jnp.float32)
            a = (jax.nn.gelu(g, approximate=True) * u).astype(jnp.bfloat16)
            y = jnp.dot(a, wd_s[...], preferred_element_type=jnp.float32)
            if X1:
                x1 = x1_s[pl.ds(r0, RB), :]
            else:
                x1 = x_s[pl.ds(r0, RB), :].astype(jnp.float32) + ga * acc_s[pl.ds(r0, RB), :]
            out_s[pl.ds(r0, RB), :] = (x1 + gb * y).astype(out_s.dtype)
            for j in range(OSPLIT):
                out_copy(r0 + j * (RB // OSPLIT), RB // OSPLIT).start()

        ln_part(0)

        def body(i, carry):
            for u in range(FUNROLL):
                ii = i * FUNROLL + u
                r0 = pl.multiple_of(ii * RB, RB)
                h2 = h_s[pl.ds(r0, RB), :]
                rn = pl.multiple_of(jnp.minimum(ii + 1, NR - 1) * RB, RB)
                ln_part(rn)
                ffn_part(r0, h2)
            return carry
        jax.lax.fori_loop(0, NR // FUNROLL, body, 0)
        pltpu.make_async_copy(out_s, out_hbm, sem_out).wait()


@jax.jit
def pallas_adaLN_cond__mha_block_cached__geglu_ffn__prompt_kernel(A_x, A_k_cache, A_v_cache, A_wq, A_wo, B_x, B_w_gate, B_w_up, B_w_down, c, w_mod):
    x = A_x.reshape(S, D)
    k = A_k_cache.reshape(H, SK, DH)
    v = A_v_cache.reshape(H, SK, DH)
    anyspec = pl.BlockSpec(memory_space=pl.ANY)
    bf = jnp.bfloat16
    out = pl.pallas_call(
        _kernel,
        in_specs=[anyspec] * 10,
        out_specs=anyspec,
        out_shape=jax.ShapeDtypeStruct((S, D), bf),
        scratch_shapes=[
            pltpu.VMEM((S, D), bf),
            pltpu.VMEM((H, D + 2 * SK, DH), bf),
            pltpu.VMEM((H, DH, D), bf),
            pltpu.VMEM((D, F), bf),
            pltpu.VMEM((D, F), bf),
            pltpu.VMEM((F, D), bf),
            pltpu.VMEM((1, D), bf),
            pltpu.VMEM((D, 6 * D), bf),
            pltpu.VMEM((S, D), bf),
            pltpu.VMEM((S, D), jnp.float32),
            pltpu.VMEM((S, D), jnp.float32),
            pltpu.VMEM((BQ, DH), bf),
            pltpu.VMEM((S, D), bf),
            pltpu.SemaphoreType.DMA((2,)),
            pltpu.SemaphoreType.DMA((NX,)),
            pltpu.SemaphoreType.DMA((H,)),
            pltpu.SemaphoreType.DMA((4,)),
            pltpu.SemaphoreType.DMA((4,)),
            pltpu.SemaphoreType.DMA(()),
        ],
        compiler_params=pltpu.CompilerParams(
            vmem_limit_bytes=100 * 1024 * 1024, flags=FLAGS,
            disable_bounds_checks=bool(NOBC), disable_semaphore_checks=bool(NOSC),
        ),
    )(x, k, v, A_wq, A_wo, B_w_gate, B_w_up, B_w_down, c, w_mod)
    return out.reshape(1, S, D)
```

```python
import jax
import jax.numpy as jnp
import jax.experimental.pallas as pl
import jax.experimental.pallas.tpu as pltpu

S, D, H, SK, DH, F = 2048, 512, 32, 2048, 128, 1792
BQ = 256
G = 512
NG = SK // G
NB = S // BQ
QSCALE = DH ** -0.5 * 1.4426950408889634
BATCH1, BATCH2 = (4, 12, 24), (12, 24, H)


def _ln(x):
    m = jnp.mean(x, axis=-1, keepdims=True)
    xc = x - m
    v = jnp.mean(xc * xc, axis=-1, keepdims=True)
    return xc * jax.lax.rsqrt(v + 1e-5)


def _tiles(s):
    return [s[:, t * 128:(t + 1) * 128] for t in range(s.shape[1] // 128)]


def _tree(f, xs):
    while len(xs) > 1:
        xs = [f(xs[i], xs[i + 1]) if i + 1 < len(xs) else xs[i] for i in range(0, len(xs), 2)]
    return xs[0]


def _dot(a, b):
    return jnp.dot(a, b, preferred_element_type=jnp.float32)


def _kernel(x_hbm, k_hbm, v_hbm, wq_hbm, wo_hbm, wg_hbm, wu_hbm, wd_hbm, c_hbm, wmod_hbm,
            out_hbm,
            x_s, kvq_s, wo_s, wg_s, wu_s, wd_s, c_s, wmod_s, h_s, acc_s, olast_s, out_s,
            sem_c, sem_x, sem_kvq, sem_h0, sem_w, sem_out):

    c_copy = pltpu.make_async_copy(c_hbm, c_s, sem_c.at[0])
    moda_copy = pltpu.make_async_copy(wmod_hbm.at[:, 0:2 * D], wmod_s.at[:, 0:2 * D], sem_c.at[1])
    x_copies = [pltpu.make_async_copy(x_hbm.at[b * BQ:(b + 1) * BQ, :], x_s.at[b * BQ:(b + 1) * BQ, :],
                                      sem_x.at[b]) for b in range(NB)]
    w_copies = [pltpu.make_async_copy(wmod_hbm.at[:, 2 * D:], wmod_s.at[:, 2 * D:], sem_w.at[0]),
                pltpu.make_async_copy(wg_hbm, wg_s, sem_w.at[1]),
                pltpu.make_async_copy(wu_hbm, wu_s, sem_w.at[2]),
                pltpu.make_async_copy(wd_hbm, wd_s, sem_w.at[3])]

    def head_copies(h, sems=None):
        c0 = h * DH if isinstance(h, int) else pl.multiple_of(h * DH, DH)
        sm = [sem_kvq.at[h]] * 4 if sems is None else sems
        return (pltpu.make_async_copy(wq_hbm.at[:, pl.ds(c0, DH)], kvq_s.at[h, pl.ds(0, D)], sm[0]),
                pltpu.make_async_copy(k_hbm.at[h], kvq_s.at[h, pl.ds(D, SK)], sm[1]),
                pltpu.make_async_copy(v_hbm.at[h], kvq_s.at[h, pl.ds(D + SK, SK)], sm[2]),
                pltpu.make_async_copy(wo_hbm.at[pl.ds(c0, DH), :], wo_s.at[h], sm[3]))

    def out_copy(r0, n):
        r0 = pl.multiple_of(r0, n)
        return pltpu.make_async_copy(out_s.at[pl.ds(r0, n), :], out_hbm.at[pl.ds(r0, n), :], sem_out)

    wq0, k0, v0, wo0 = head_copies(0, [sem_h0.at[i] for i in range(4)])
    first = [c_copy, moda_copy, x_copies[0], x_copies[1], wq0, k0, v0, x_copies[2], x_copies[3], wo0]
    first += x_copies[4:]

    def start_first(i, carry):
        for k, cp in enumerate(first):
            pl.when(i == k)(cp.start)
        return carry
    jax.lax.fori_loop(0, len(first), start_first, 0)

    def start_head(h, carry):
        for cp in head_copies(h):
            cp.start()
        return carry + 1
    n_started = jax.lax.fori_loop(1, BATCH1[1], start_head, 0)

    acc_s[(NB - 1) * BQ:, :] = jnp.zeros((BQ, D), jnp.float32)
    c_copy.wait()
    moda_copy.wait()
    c = c_s[...].astype(jnp.float32)
    sc = jnp.broadcast_to((c * jax.nn.sigmoid(c)).astype(jnp.bfloat16), (16, D))
    moda = _dot(sc, wmod_s[:, 0:2 * D])[0:1]
    sa = moda[:, 0:D]
    ca1 = 1.0 + moda[:, D:2 * D]

    def run_head(h, never, is_first):
        def KK(b): return [('K', b, g) for g in range(NG)]
        def PP(b): return [('P', b, g) for g in range(NG)]
        if is_first:
            stages = [('W', x_copies[0], x_copies[1], wq0), ('L', 0), ('L', 1), ('Q', 0), ('Q', 1), ('W', k0)]
            stages += KK(0) + KK(1) + [('W', v0, x_copies[2], x_copies[3], wo0), ('L', 2), ('L', 3)]
            stages += PP(0) + [('Q', 2)] + KK(2) + [('O', 0), ('Q', 3)] + PP(1) + KK(3)
            stages += [('W', *x_copies[4:]), ('L', 4), ('L', 5), ('L', 6), ('L', 7), ('O', 1)] + PP(2)
            stages += [('Q', 4)] + KK(4) + [('O', 2), ('Q', 5)] + PP(3) + KK(5)
            stages += [('O', 3), ('Q', 6)] + PP(4) + KK(6) + [('O', 4), ('Q', 7)] + PP(5) + KK(7)
            stages += [('O', 5)] + PP(6) + [('O', 6)] + PP(7)
        else:
            stages = [('Q', 0), ('Q', 1)] + KK(0)
            for b in range(NB):
                if b + 1 < NB:
                    stages += KK(b + 1)
                stages += [('O', b - 1)]
                if b + 2 < NB:
                    stages += [('Q', b + 2)]
                stages += PP(b)

        q, ss, mx, l, acc, onorm, hq = {}, {}, {}, {}, {}, {}, {}
        prev = None
        for st in stages:
            kind = st[0]
            if kind == 'W':
                for cp in st[1:]:
                    cp.wait()
            elif kind == 'L':
                b = st[1]
                xx = x_s[b * BQ:(b + 1) * BQ, :].astype(jnp.float32)
                hq[b] = (_ln(xx) * ca1 + sa).astype(jnp.bfloat16)
                h_s[b * BQ:(b + 1) * BQ, :] = hq[b]
            elif kind == 'Q':
                b = st[1]
                qf = _dot(hq[b] if is_first else h_s[b * BQ:(b + 1) * BQ, :], kvq_s[h, 0:D, :])
                q[b] = (qf * QSCALE).astype(jnp.bfloat16)
                prev = qf
            elif kind == 'K':
                _, b, g = st
                s = jax.lax.dot_general(q[b], kvq_s[h, D + g * G:D + (g + 1) * G, :],
                                        (((1,), (1,)), ((), ())), preferred_element_type=jnp.float32)
                ss[b, g] = s
                prev = s[:, 0:128]
                if g == NG - 1:
                    mm = _tree(jnp.maximum, [t for gg in range(NG) for t in _tiles(ss[b, gg])])
                    mx[b] = jnp.broadcast_to(jnp.max(mm, axis=-1, keepdims=True), (BQ, 128))
            elif kind == 'O':
                b = st[1]
                if b < 0:
                    b = NB - 1
                    y = _dot(olast_s[...], wo_s[jnp.maximum(h - 1, 0)])
                else:
                    y = _dot(onorm[b], wo_s[h])
                if is_first:
                    acc_s[b * BQ:(b + 1) * BQ, :] = y
                else:
                    acc_s[b * BQ:(b + 1) * BQ, :] += y
                prev = y[:, 0:128]
            else:
                _, b, g = st
                m = jnp.where(never, prev, mx[b])
                ts = [jnp.exp2(t - m) for t in _tiles(ss[b, g])]
                dl = _tree(jnp.add, ts)
                l[b] = dl if g == 0 else l[b] + dl
                ts[-1] = jnp.where(never, l[b], ts[-1])
                p = jnp.concatenate(ts, axis=1).astype(jnp.bfloat16)
                do = _dot(p, kvq_s[h, D + SK + g * G:D + SK + (g + 1) * G, :])
                acc[b] = do if g == 0 else acc[b] + do
                prev = do
                if g == NG - 1:
                    lsum = jnp.sum(l[b], axis=-1, keepdims=True)
                    r = pl.reciprocal(lsum, approx=True)
                    r = r * (2.0 - lsum * r)
                    onorm[b] = (acc[b] * r).astype(jnp.bfloat16)
                    if b == NB - 1:
                        olast_s[...] = onorm[b]

    run_head(0, n_started > 1000, True)

    def head_body(h, carry):
        for cp in head_copies(h):
            cp.wait()

        for batch in (BATCH1, BATCH2):
            @pl.when(h == batch[0])
            def _(batch=batch):
                for hh in range(batch[1], batch[2]):
                    for cp in head_copies(hh):
                        cp.start()
                if batch is BATCH2:
                    for cp in w_copies:
                        cp.start()

        run_head(h, h > 1000, False)
        return carry

    jax.lax.fori_loop(1, H, head_body, 0)

    for cp in w_copies:
        cp.wait()
    acc_s[(NB - 1) * BQ:, :] += _dot(olast_s[...], wo_s[H - 1])
    modb = _dot(sc, wmod_s[:, 2 * D:])[0:1]
    ga = modb[:, 0:D]
    sb = modb[:, D:2 * D]
    cb1 = 1.0 + modb[:, 2 * D:3 * D]
    gb = modb[:, 3 * D:4 * D]

    def resid(rows):
        return x_s[rows, :].astype(jnp.float32) + ga * acc_s[rows, :]

    def ln_part(rows):
        hf = _ln(resid(rows)) * cb1 + sb
        h_s[rows, :] = hf.astype(jnp.bfloat16)
        return hf

    def ffn_part(r0, rn, never):
        rows = pl.ds(r0, BQ)
        h2 = h_s[rows, :]
        g = _dot(h2, wg_s[...])
        hf = ln_part(pl.ds(rn, BQ))
        u = _dot(h2, wu_s[...])
        ts = _tiles(jax.nn.gelu(g, approximate=True) * u)
        for t, ht in enumerate(_tiles(hf)):
            ts[t] = jnp.where(never, ht, ts[t])
        a = jnp.concatenate(ts, axis=1).astype(jnp.bfloat16)
        y = _dot(a, wd_s[...])
        out_s[rows, :] = (resid(rows) + gb * y).astype(out_s.dtype)
        for j in range(2):
            out_copy(r0 + j * (BQ // 2), BQ // 2).start()

    ln_part(pl.ds(0, BQ))

    def ffn_body(i, carry):
        for k in range(2):
            ii = i * 2 + k
            r0 = pl.multiple_of(ii * BQ, BQ)
            rn = pl.multiple_of(jnp.minimum(ii + 1, NB - 1) * BQ, BQ)
            ffn_part(r0, rn, i > 1000)
        return carry
    jax.lax.fori_loop(0, NB // 2, ffn_body, 0)
    pltpu.make_async_copy(out_s, out_hbm, sem_out).wait()


@jax.jit
def pallas_adaLN_cond__mha_block_cached__geglu_ffn__prompt_kernel(
    A_x: jax.Array,
    A_k_cache: jax.Array,
    A_v_cache: jax.Array,
    A_wq: jax.Array,
    A_wo: jax.Array,
    B_x: jax.Array,
    B_w_gate: jax.Array,
    B_w_up: jax.Array,
    B_w_down: jax.Array,
    c: jax.Array,
    w_mod: jax.Array,
):
    del B_x
    hbm = pl.BlockSpec(memory_space=pl.ANY)
    bf = jnp.bfloat16
    out = pl.pallas_call(
        _kernel,
        in_specs=[hbm] * 10,
        out_specs=hbm,
        out_shape=jax.ShapeDtypeStruct((S, D), bf),
        scratch_shapes=[
            pltpu.VMEM((S, D), bf),
            pltpu.VMEM((H, D + 2 * SK, DH), bf),
            pltpu.VMEM((H, DH, D), bf),
            pltpu.VMEM((D, F), bf),
            pltpu.VMEM((D, F), bf),
            pltpu.VMEM((F, D), bf),
            pltpu.VMEM((1, D), bf),
            pltpu.VMEM((D, 6 * D), bf),
            pltpu.VMEM((S, D), bf),
            pltpu.VMEM((S, D), jnp.float32),
            pltpu.VMEM((BQ, DH), bf),
            pltpu.VMEM((S, D), bf),
            pltpu.SemaphoreType.DMA((2,)),
            pltpu.SemaphoreType.DMA((NB,)),
            pltpu.SemaphoreType.DMA((H,)),
            pltpu.SemaphoreType.DMA((4,)),
            pltpu.SemaphoreType.DMA((4,)),
            pltpu.SemaphoreType.DMA(()),
        ],
        compiler_params=pltpu.CompilerParams(
            vmem_limit_bytes=100 * 1024 * 1024,
            disable_bounds_checks=True,
            disable_semaphore_checks=True,
        ),
    )(A_x.reshape(S, D), A_k_cache.reshape(H, SK, DH), A_v_cache.reshape(H, SK, DH),
      A_wq, A_wo, B_w_gate, B_w_up, B_w_down, c, w_mod)
    return out.reshape(1, S, D)
```

```python
import jax
import jax.numpy as jnp
import jax.experimental.pallas as pl
import jax.experimental.pallas.tpu as pltpu

S, D, H, SK, DH, F = 2048, 512, 32, 2048, 128, 1792
BQ = 256
G = 512
NG = SK // G
NB = S // BQ
QSCALE = DH ** -0.5 * 1.4426950408889634
LOOK = 3
RING = LOOK + 1
PADR = 16
NPAD = 8


def _ln(x):
    m = jnp.mean(x, axis=-1, keepdims=True)
    xc = x - m
    v = jnp.mean(xc * xc, axis=-1, keepdims=True)
    return xc * jax.lax.rsqrt(v + 1e-5)


def _tiles(s):
    return [s[:, t * 128:(t + 1) * 128] for t in range(s.shape[1] // 128)]


def _tree(f, xs):
    while len(xs) > 1:
        xs = [f(xs[i], xs[i + 1]) if i + 1 < len(xs) else xs[i] for i in range(0, len(xs), 2)]
    return xs[0]


def _dot(a, b):
    return jnp.dot(a, b, preferred_element_type=jnp.float32)


def _dot_nt(a, b):
    return jax.lax.dot_general(a, b, (((1,), (1,)), ((), ())), preferred_element_type=jnp.float32)


def _rows(b):
    return slice(b * BQ, (b + 1) * BQ)


def _kk(b, gs=range(NG)):
    return [('K', b, g) for g in gs]


def _pp(b, gs=range(NG)):
    return [('P', b, g) for g in gs]


def _first_head_plan():
    st = [('W', 'x0', 'wq'), ('L', 0), ('Q', 0), ('W', 'k')]
    st += _kk(0, (0, 1)) + [('W', 'x1'), ('L', 1)] + _kk(0, (2, 3)) + [('Q', 1)] + _kk(1) + [('W', 'v')]
    st += _pp(0, (0, 1)) + [('W', 'x2'), ('L', 2)] + _pp(0, (2, 3)) + [('Q', 2)]
    st += _kk(2, (0, 1, 2)) + [('W', 'wo')] + _kk(2, (3,)) + [('O', 0)]
    st += _pp(1, (0, 1)) + [('W', 'x3', 'x4', 'x5', 'x6', 'x7'), ('L', 3)] + _pp(1, (2, 3))
    for b in range(2, NB - 2):
        st += [('Q', b + 1)] + _kk(b + 1) + [('O', b - 1)] + _pp(b, (0, 1)) + [('L', b + 2)] + _pp(b, (2, 3))
    for b in range(NB - 2, NB):
        if b + 1 < NB:
            st += [('Q', b + 1)] + _kk(b + 1)
        st += [('O', b - 1)] + _pp(b)
    return st


def _head_plan():
    st = [('Q', 0), ('Q', 1)] + _kk(0)
    for b in range(NB):
        if b + 1 < NB:
            st += _kk(b + 1)
        st += [('O', b - 1)]
        if b + 2 < NB:
            st += [('Q', b + 2)]
        st += _pp(b)
    return st


FIRST_STAGES = _first_head_plan()
WAIT_GROUPS = [st[1:] for st in FIRST_STAGES if st[0] == 'W']
GROUP_OF = {name: i for i, grp in enumerate(WAIT_GROUPS) for name in grp}


def _kernel(x_hbm, k_hbm, v_hbm, wq_hbm, wo_hbm, wg_hbm, wu_hbm, wd_hbm, c_hbm, wmod_hbm,
            out_hbm,
            x_s, kvq_s, wo_s, wg_s, wu_s, wd_s, c_s, wmod_s, h_s, acc_s, olast_s, out_s,
            sem_c, sem_g, sem_k, sem_w, sem_out):

    c_copy = pltpu.make_async_copy(c_hbm, c_s, sem_c)
    moda_copy = pltpu.make_async_copy(wmod_hbm.at[:, 0:2 * D], wmod_s.at[:, 0:2 * D], sem_c)
    w_copies = [pltpu.make_async_copy(wmod_hbm.at[:, 2 * D:], wmod_s.at[:, 2 * D:], sem_w),
                pltpu.make_async_copy(wg_hbm, wg_s, sem_w),
                pltpu.make_async_copy(wu_hbm, wu_s, sem_w),
                pltpu.make_async_copy(wd_hbm, wd_s, sem_w)]

    def head_copies(h, sems=None):
        c0 = h * DH if isinstance(h, int) else pl.multiple_of(h * DH, DH)
        sm = [sem_k.at[h & (RING - 1)]] * 4 if sems is None else sems
        return [pltpu.make_async_copy(wq_hbm.at[:, pl.ds(c0, DH)], kvq_s.at[h, pl.ds(0, D)], sm[0]),
                pltpu.make_async_copy(k_hbm.at[h], kvq_s.at[h, pl.ds(D, SK)], sm[1]),
                pltpu.make_async_copy(v_hbm.at[h], kvq_s.at[h, pl.ds(D + SK, SK)], sm[2]),
                pltpu.make_async_copy(wo_hbm.at[pl.ds(c0, DH), :], wo_s.at[h], sm[3])]

    first = {f'x{b}': pltpu.make_async_copy(x_hbm.at[_rows(b), :], x_s.at[_rows(b), :], sem_g.at[GROUP_OF[f'x{b}']])
             for b in range(NB)}
    first['wq'], first['k'], first['v'], first['wo'] = head_copies(
        0, [sem_g.at[GROUP_OF[n]] for n in ('wq', 'k', 'v', 'wo')])

    def out_copy(r0, n):
        r0 = pl.multiple_of(r0, n)
        return pltpu.make_async_copy(out_s.at[pl.ds(r0, n), :], out_hbm.at[pl.ds(r0, n), :], sem_out)

    early = [c_copy, moda_copy] + [first[n] for n in
                                   ('x0', 'wq', 'k', 'x1', 'v', 'x2', 'wo', 'x3', 'x4', 'x5', 'x6', 'x7')]

    def start_early(i, carry):
        for k, cp in enumerate(early):
            pl.when(i == k)(cp.start)
        return carry
    jax.lax.fori_loop(0, len(early), start_early, 0)

    def start_head(h, carry):
        for cp in head_copies(h):
            cp.start()
        return carry + 1
    n_started = jax.lax.fori_loop(1, LOOK + 1, start_head, 0)

    acc_s[_rows(NB - 1), :] = jnp.zeros((BQ, D), jnp.float32)
    c_copy.wait()
    moda_copy.wait()
    c = c_s[...].astype(jnp.float32)
    sc = jnp.broadcast_to((c * jax.nn.sigmoid(c)).astype(jnp.bfloat16), (16, D))
    moda = _dot(sc, wmod_s[:, 0:2 * D])[0:1]
    sa = moda[:, 0:D]
    ca1 = 1.0 + moda[:, D:2 * D]

    kvq32 = kvq_s.bitcast(jnp.uint32)

    def ld(h, r0, n):
        return pltpu.bitcast(kvq32[h, r0 // 2:(r0 + n) // 2, :], jnp.bfloat16)

    def anchor(slot, names, val):
        r0 = PADR * (slot % NPAD)
        pads = {'x': x_s.at[pl.ds(S + r0, PADR), 0:128], 'kvq': kvq_s.at[H, pl.ds(r0, PADR), :],
                'wo': wo_s.at[H, pl.ds(r0, PADR), 0:128]}
        for buf in sorted({'x' if n[0] == 'x' else ('wo' if n == 'wo' else 'kvq') for n in names}):
            pads[buf][...] = val[0:PADR, :].astype(jnp.bfloat16)

    def run_head(h, stages, first_head, never):
        q, hq, ss, mx, l, acc, onorm = {}, {}, {}, {}, {}, {}, {}
        prev = jnp.broadcast_to(sa[:, 0:128], (PADR, 128)) if first_head else None
        n_waits = 0
        for st in stages:
            kind = st[0]
            if kind == 'W':
                anchor(n_waits, st[1:], prev)
                n_waits += 1
                for name in st[1:]:
                    first[name].wait()
            elif kind == 'L':
                b = st[1]
                hq[b] = (_ln(x_s[_rows(b), :].astype(jnp.float32)) * ca1 + sa).astype(jnp.bfloat16)
                h_s[_rows(b), :] = hq[b]
            elif kind == 'Q':
                b = st[1]
                prev = _dot(hq[b] if first_head else h_s[_rows(b), :], ld(h, 0, D))
                q[b] = (prev * QSCALE).astype(jnp.bfloat16)
            elif kind == 'K':
                _, b, g = st
                ss[b, g] = _dot_nt(q[b], ld(h, D + g * G, G))
                prev = ss[b, g][:, 0:128]
                if g == NG - 1:
                    mm = _tree(jnp.maximum, [t for gg in range(NG) for t in _tiles(ss[b, gg])])
                    mx[b] = jnp.broadcast_to(jnp.max(mm, axis=-1, keepdims=True), (BQ, 128))
            elif kind == 'O':
                b = st[1]
                if b < 0:
                    b = NB - 1
                    y = _dot(olast_s[...], wo_s[h - 1])
                else:
                    y = _dot(onorm[b], wo_s[h])
                if first_head:
                    acc_s[_rows(b), :] = y
                else:
                    acc_s[_rows(b), :] += y
                prev = y[:, 0:128]
            else:
                _, b, g = st
                m = jnp.where(never, prev, mx[b])
                ts = [jnp.exp2(t - m) for t in _tiles(ss[b, g])]
                dl = _tree(jnp.add, ts)
                l[b] = dl if g == 0 else l[b] + dl
                ts[-1] = jnp.where(never, l[b], ts[-1])
                p = jnp.concatenate(ts, axis=1).astype(jnp.bfloat16)
                prev = _dot(p, ld(h, D + SK + g * G, G))
                acc[b] = prev if g == 0 else acc[b] + prev
                if g == NG - 1:
                    lsum = jnp.sum(l[b], axis=-1, keepdims=True)
                    r = pl.reciprocal(lsum, approx=True)
                    r = r * (2.0 - lsum * r)
                    onorm[b] = (acc[b] * r).astype(jnp.bfloat16)
                    if b == NB - 1:
                        olast_s[...] = onorm[b]

    run_head(0, FIRST_STAGES, True, n_started > 1000)

    def head_body(h, carry):
        for cp in head_copies(h):
            cp.wait()

        @pl.when(h + LOOK < H)
        def _():
            for cp in head_copies(jnp.minimum(h + LOOK, H - 1)):
                cp.start()

        @pl.when(h == H - LOOK)
        def _():
            for cp in w_copies:
                cp.start()

        run_head(h, _head_plan(), False, h > 1000)
        return carry

    jax.lax.fori_loop(1, H, head_body, 0)

    for cp in w_copies:
        cp.wait()
    acc_s[_rows(NB - 1), :] += _dot(olast_s[...], wo_s[H - 1])
    modb = _dot(sc, wmod_s[:, 2 * D:])[0:1]
    ga = modb[:, 0:D]
    sb = modb[:, D:2 * D]
    cb1 = 1.0 + modb[:, 2 * D:3 * D]
    gb = modb[:, 3 * D:4 * D]

    def resid(rows):
        return x_s[rows, :].astype(jnp.float32) + ga * acc_s[rows, :]

    def ln_part(rows):
        hf = _ln(resid(rows)) * cb1 + sb
        h_s[rows, :] = hf.astype(jnp.bfloat16)
        return hf

    def ffn_part(r0, rn, never):
        rows = pl.ds(r0, BQ)
        h2 = h_s[rows, :]
        g = _dot(h2, wg_s[...])
        hf = ln_part(pl.ds(rn, BQ))
        u = _dot(h2, wu_s[...])
        ts = _tiles(jax.nn.gelu(g, approximate=True) * u)
        for t, ht in enumerate(_tiles(hf)):
            ts[t] = jnp.where(never, ht, ts[t])
        a = jnp.concatenate(ts, axis=1).astype(jnp.bfloat16)
        y = _dot(a, wd_s[...])
        out_s[rows, :] = (resid(rows) + gb * y).astype(out_s.dtype)
        for j in range(2):
            out_copy(r0 + j * (BQ // 2), BQ // 2).start()

    ln_part(pl.ds(0, BQ))

    def ffn_body(i, carry):
        for k in range(2):
            ii = i * 2 + k
            r0 = pl.multiple_of(ii * BQ, BQ)
            rn = pl.multiple_of(jnp.minimum(ii + 1, NB - 1) * BQ, BQ)
            ffn_part(r0, rn, i > 1000)
        return carry
    jax.lax.fori_loop(0, NB // 2, ffn_body, 0)
    pltpu.make_async_copy(out_s, out_hbm, sem_out).wait()


@jax.jit
def pallas_adaLN_cond__mha_block_cached__geglu_ffn__prompt_kernel(
    A_x: jax.Array,
    A_k_cache: jax.Array,
    A_v_cache: jax.Array,
    A_wq: jax.Array,
    A_wo: jax.Array,
    B_x: jax.Array,
    B_w_gate: jax.Array,
    B_w_up: jax.Array,
    B_w_down: jax.Array,
    c: jax.Array,
    w_mod: jax.Array,
):
    del B_x
    hbm = pl.BlockSpec(memory_space=pl.ANY)
    bf = jnp.bfloat16
    out = pl.pallas_call(
        _kernel,
        in_specs=[hbm] * 10,
        out_specs=hbm,
        out_shape=jax.ShapeDtypeStruct((S, D), bf),
        scratch_shapes=[
            pltpu.VMEM((S + PADR * NPAD, D), bf),
            pltpu.VMEM((H + 1, D + 2 * SK, DH), bf),
            pltpu.VMEM((H + 1, DH, D), bf),
            pltpu.VMEM((D, F), bf),
            pltpu.VMEM((D, F), bf),
            pltpu.VMEM((F, D), bf),
            pltpu.VMEM((1, D), bf),
            pltpu.VMEM((D, 6 * D), bf),
            pltpu.VMEM((S, D), bf),
            pltpu.VMEM((S, D), jnp.float32),
            pltpu.VMEM((BQ, DH), bf),
            pltpu.VMEM((S, D), bf),
            pltpu.SemaphoreType.DMA(()),
            pltpu.SemaphoreType.DMA((len(WAIT_GROUPS),)),
            pltpu.SemaphoreType.DMA((RING,)),
            pltpu.SemaphoreType.DMA(()),
            pltpu.SemaphoreType.DMA(()),
        ],
        compiler_params=pltpu.CompilerParams(
            vmem_limit_bytes=100 * 1024 * 1024,
            flags={"XLA_TPU_RESCHEDULE_DMA_DONES": True},
        ),
    )(A_x.reshape(S, D), A_k_cache.reshape(H, SK, DH), A_v_cache.reshape(H, SK, DH),
      A_wq, A_wo, B_w_gate, B_w_up, B_w_down, c, w_mod)
    return out.reshape(1, S, D)
```

```python
import jax
import jax.numpy as jnp
import jax.experimental.pallas as pl
import jax.experimental.pallas.tpu as pltpu

S, D, H, SK, DH, F = 2048, 512, 32, 2048, 128, 1792
BQ = 256
G = 512
NG = SK // G
NB = S // BQ
QSCALE = DH ** -0.5 * 1.4426950408889634
LOOK = 3
RING = LOOK + 1
PADR = 16
NPAD = 8


def _ln(x):
    m = jnp.mean(x, axis=-1, keepdims=True)
    xc = x - m
    v = jnp.mean(xc * xc, axis=-1, keepdims=True)
    return xc * jax.lax.rsqrt(v + 1e-5)


def _tiles(s):
    return [s[:, t * 128:(t + 1) * 128] for t in range(s.shape[1] // 128)]


def _tree(f, xs):
    while len(xs) > 1:
        xs = [f(xs[i], xs[i + 1]) if i + 1 < len(xs) else xs[i] for i in range(0, len(xs), 2)]
    return xs[0]


def _dot(a, b):
    return jnp.dot(a, b, preferred_element_type=jnp.float32)


def _dot_nt(a, b):
    return jax.lax.dot_general(a, b, (((1,), (1,)), ((), ())), preferred_element_type=jnp.float32)


def _rows(b):
    return slice(b * BQ, (b + 1) * BQ)


def _kk(b, gs=range(NG)):
    return [('K', b, g) for g in gs]


def _pp(b, gs=range(NG)):
    return [('P', b, g) for g in gs]


def _first_head_plan():
    st = [('W', 'x0', 'wq'), ('L', 0), ('Q', 0), ('W', 'ka')]
    st += _kk(0, (0, 1)) + [('W', 'kb')] + _kk(0, (2,)) + [('W', 'x1'), ('L', 1)] + _kk(0, (3,))
    st += [('Q', 1)] + _kk(1) + [('W', 'v')]
    st += _pp(0, (0, 1)) + [('W', 'x2'), ('L', 2)] + _pp(0, (2, 3)) + [('Q', 2)]
    st += _kk(2, (0, 1, 2)) + [('W', 'wo')] + _kk(2, (3,)) + [('O', 0)]
    st += _pp(1, (0,)) + [('W', 'x3', 'x4', 'x5', 'x6', 'x7'), ('L', 3)] + _pp(1, (1, 2, 3))
    for b in range(2, NB - 2):
        st += [('Q', b + 1)] + _kk(b + 1, (0,)) + [('L', b + 2)] + _kk(b + 1, (1, 2, 3))
        st += [('O', b - 1)] + _pp(b)
    st += [('Q', NB - 1)] + _kk(NB - 1) + [('O', NB - 3)] + _pp(NB - 2)
    st += [('O', NB - 2)] + _pp(NB - 1)
    return st


def _head_plan():
    st = [('Q', 0), ('Q', 1)] + _kk(0)
    for b in range(NB):
        if b + 1 < NB:
            st += _kk(b + 1)
        st += [('O', b - 1)]
        if b + 2 < NB:
            st += [('Q', b + 2)]
        st += _pp(b)
    return st


FIRST_STAGES = _first_head_plan()
WAIT_GROUPS = [st[1:] for st in FIRST_STAGES if st[0] == 'W']
GROUP_OF = {name: i for i, grp in enumerate(WAIT_GROUPS) for name in grp}


def _kernel(x_hbm, k_hbm, v_hbm, wq_hbm, wo_hbm, wg_hbm, wu_hbm, wd_hbm, c_hbm, wmod_hbm,
            out_hbm,
            x_s, kvq_s, wo_s, wg_s, wu_s, wd_s, c_s, wmod_s, h_s, acc_s, olast_s, out_s,
            sem_c, sem_g, sem_k, sem_w, sem_out):

    c_copy = pltpu.make_async_copy(c_hbm, c_s, sem_c)
    moda_copy = pltpu.make_async_copy(wmod_hbm.at[:, 0:2 * D], wmod_s.at[:, 0:2 * D], sem_c)
    w_copies = [pltpu.make_async_copy(wmod_hbm.at[:, 2 * D:], wmod_s.at[:, 2 * D:], sem_w),
                pltpu.make_async_copy(wg_hbm, wg_s, sem_w),
                pltpu.make_async_copy(wu_hbm, wu_s, sem_w),
                pltpu.make_async_copy(wd_hbm, wd_s, sem_w)]

    def head_copies(h):
        c0 = pl.multiple_of(h * DH, DH)
        sem = sem_k.at[h & (RING - 1)]
        return [pltpu.make_async_copy(wq_hbm.at[:, pl.ds(c0, DH)], kvq_s.at[h, pl.ds(0, D)], sem),
                pltpu.make_async_copy(k_hbm.at[h], kvq_s.at[h, pl.ds(D, SK)], sem),
                pltpu.make_async_copy(v_hbm.at[h], kvq_s.at[h, pl.ds(D + SK, SK)], sem),
                pltpu.make_async_copy(wo_hbm.at[pl.ds(c0, DH), :], wo_s.at[h], sem)]

    first = {f'x{b}': pltpu.make_async_copy(x_hbm.at[_rows(b), :], x_s.at[_rows(b), :], sem_g.at[GROUP_OF[f'x{b}']])
             for b in range(NB)}
    first['wq'] = pltpu.make_async_copy(wq_hbm.at[:, pl.ds(0, DH)], kvq_s.at[0, pl.ds(0, D)], sem_g.at[GROUP_OF['wq']])
    for name, r0 in (('ka', 0), ('kb', SK // 2)):
        first[name] = pltpu.make_async_copy(k_hbm.at[0, pl.ds(r0, SK // 2)], kvq_s.at[0, pl.ds(D + r0, SK // 2)],
                                            sem_g.at[GROUP_OF[name]])
    first['v'] = pltpu.make_async_copy(v_hbm.at[0], kvq_s.at[0, pl.ds(D + SK, SK)], sem_g.at[GROUP_OF['v']])
    first['wo'] = pltpu.make_async_copy(wo_hbm.at[pl.ds(0, DH), :], wo_s.at[0], sem_g.at[GROUP_OF['wo']])

    def out_copy(r0, n):
        r0 = pl.multiple_of(r0, n)
        return pltpu.make_async_copy(out_s.at[pl.ds(r0, n), :], out_hbm.at[pl.ds(r0, n), :], sem_out)

    early = [c_copy, moda_copy] + [first[n] for n in
                                   ('x0', 'wq', 'ka', 'kb', 'x1', 'v', 'x2', 'wo', 'x3', 'x4', 'x5', 'x6', 'x7')]

    def start_early(i, carry):
        for k, cp in enumerate(early):
            pl.when(i == k)(cp.start)
        return carry
    jax.lax.fori_loop(0, len(early), start_early, 0)

    def start_head(h, carry):
        for cp in head_copies(h):
            cp.start()
        return carry + 1
    n_started = jax.lax.fori_loop(1, LOOK + 1, start_head, 0)

    acc_s[_rows(NB - 1), :] = jnp.zeros((BQ, D), jnp.float32)
    c_copy.wait()
    moda_copy.wait()
    c = c_s[...].astype(jnp.float32)
    sc = jnp.broadcast_to((c * jax.nn.sigmoid(c)).astype(jnp.bfloat16), (16, D))
    moda = _dot(sc, wmod_s[:, 0:2 * D])[0:1]
    sa = moda[:, 0:D]
    ca1 = 1.0 + moda[:, D:2 * D]

    kvq32 = kvq_s.bitcast(jnp.uint32)

    def ld(h, r0, n):
        return pltpu.bitcast(kvq32[h, r0 // 2:(r0 + n) // 2, :], jnp.bfloat16)

    def anchor(slot, names, val):
        r0 = PADR * (slot % NPAD)
        pads = {'x': x_s.at[pl.ds(S + r0, PADR), 0:128], 'kvq': kvq_s.at[H, pl.ds(r0, PADR), :],
                'wo': wo_s.at[H, pl.ds(r0, PADR), 0:128]}
        for buf in sorted({'x' if n[0] == 'x' else ('wo' if n == 'wo' else 'kvq') for n in names}):
            pads[buf][...] = val[0:PADR, :].astype(jnp.bfloat16)

    def run_head(h, stages, first_head, never):
        q, hq, ss, mx, l, acc, onorm = {}, {}, {}, {}, {}, {}, {}
        prev = jnp.broadcast_to(sa[:, 0:128], (PADR, 128)) if first_head else None
        n_waits = 0
        for st in stages:
            kind = st[0]
            if kind == 'W':
                anchor(n_waits, st[1:], prev)
                n_waits += 1
                for name in st[1:]:
                    first[name].wait()
            elif kind == 'L':
                b = st[1]
                hq[b] = (_ln(x_s[_rows(b), :].astype(jnp.float32)) * ca1 + sa).astype(jnp.bfloat16)
                h_s[_rows(b), :] = hq[b]
            elif kind == 'Q':
                b = st[1]
                prev = _dot(hq[b] if first_head else h_s[_rows(b), :], ld(h, 0, D))
                q[b] = (prev * QSCALE).astype(jnp.bfloat16)
            elif kind == 'K':
                _, b, g = st
                ss[b, g] = _dot_nt(q[b], ld(h, D + g * G, G))
                prev = ss[b, g][:, 0:128]
                if g == NG - 1:
                    mm = _tree(jnp.maximum, [t for gg in range(NG) for t in _tiles(ss[b, gg])])
                    mx[b] = jnp.broadcast_to(jnp.max(mm, axis=-1, keepdims=True), (BQ, 128))
            elif kind == 'O':
                b = st[1]
                if b < 0:
                    b = NB - 1
                    y = _dot(olast_s[...], wo_s[h - 1])
                else:
                    y = _dot(onorm[b], wo_s[h])
                if first_head:
                    acc_s[_rows(b), :] = y
                else:
                    acc_s[_rows(b), :] += y
                prev = y[:, 0:128]
            else:
                _, b, g = st
                m = jnp.where(never, prev, mx[b])
                ts = [jnp.exp2(t - m) for t in _tiles(ss[b, g])]
                dl = _tree(jnp.add, ts)
                l[b] = dl if g == 0 else l[b] + dl
                ts[-1] = jnp.where(never, l[b], ts[-1])
                p = jnp.concatenate(ts, axis=1).astype(jnp.bfloat16)
                prev = _dot(p, ld(h, D + SK + g * G, G))
                acc[b] = prev if g == 0 else acc[b] + prev
                if g == NG - 1:
                    lsum = jnp.sum(l[b], axis=-1, keepdims=True)
                    r = pl.reciprocal(lsum, approx=True)
                    r = r * (2.0 - lsum * r)
                    onorm[b] = (acc[b] * r).astype(jnp.bfloat16)
                    if b == NB - 1:
                        olast_s[...] = onorm[b]

    run_head(0, FIRST_STAGES, True, n_started > 1000)

    def head_body(h, carry):
        for cp in head_copies(h):
            cp.wait()

        @pl.when(h + LOOK < H)
        def _():
            for cp in head_copies(jnp.minimum(h + LOOK, H - 1)):
                cp.start()

        @pl.when(h == H - LOOK)
        def _():
            for cp in w_copies:
                cp.start()

        run_head(h, _head_plan(), False, h > 1000)
        return carry

    jax.lax.fori_loop(1, H, head_body, 0)

    for cp in w_copies:
        cp.wait()
    acc_s[_rows(NB - 1), :] += _dot(olast_s[...], wo_s[H - 1])
    modb = _dot(sc, wmod_s[:, 2 * D:])[0:1]
    ga = modb[:, 0:D]
    sb = modb[:, D:2 * D]
    cb1 = 1.0 + modb[:, 2 * D:3 * D]
    gb = modb[:, 3 * D:4 * D]

    def resid(rows):
        return x_s[rows, :].astype(jnp.float32) + ga * acc_s[rows, :]

    def ln_part(rows):
        hf = _ln(resid(rows)) * cb1 + sb
        h_s[rows, :] = hf.astype(jnp.bfloat16)
        return hf

    def ffn_part(r0, rn, never):
        rows = pl.ds(r0, BQ)
        h2 = h_s[rows, :]
        g = _dot(h2, wg_s[...])
        hf = ln_part(pl.ds(rn, BQ))
        u = _dot(h2, wu_s[...])
        ts = _tiles(jax.nn.gelu(g, approximate=True) * u)
        for t, ht in enumerate(_tiles(hf)):
            ts[t] = jnp.where(never, ht, ts[t])
        a = jnp.concatenate(ts, axis=1).astype(jnp.bfloat16)
        y = _dot(a, wd_s[...])
        out_s[rows, :] = (resid(rows) + gb * y).astype(out_s.dtype)
        for j in range(2):
            out_copy(r0 + j * (BQ // 2), BQ // 2).start()

    ln_part(pl.ds(0, BQ))

    def ffn_body(i, carry):
        for k in range(2):
            ii = i * 2 + k
            r0 = pl.multiple_of(ii * BQ, BQ)
            rn = pl.multiple_of(jnp.minimum(ii + 1, NB - 1) * BQ, BQ)
            ffn_part(r0, rn, i > 1000)
        return carry
    jax.lax.fori_loop(0, NB // 2, ffn_body, 0)
    pltpu.make_async_copy(out_s, out_hbm, sem_out).wait()


@jax.jit
def pallas_adaLN_cond__mha_block_cached__geglu_ffn__prompt_kernel(
    A_x: jax.Array,
    A_k_cache: jax.Array,
    A_v_cache: jax.Array,
    A_wq: jax.Array,
    A_wo: jax.Array,
    B_x: jax.Array,
    B_w_gate: jax.Array,
    B_w_up: jax.Array,
    B_w_down: jax.Array,
    c: jax.Array,
    w_mod: jax.Array,
):
    del B_x
    hbm = pl.BlockSpec(memory_space=pl.ANY)
    bf = jnp.bfloat16
    out = pl.pallas_call(
        _kernel,
        in_specs=[hbm] * 10,
        out_specs=hbm,
        out_shape=jax.ShapeDtypeStruct((S, D), bf),
        scratch_shapes=[
            pltpu.VMEM((S + PADR * NPAD, D), bf),
            pltpu.VMEM((H + 1, D + 2 * SK, DH), bf),
            pltpu.VMEM((H + 1, DH, D), bf),
            pltpu.VMEM((D, F), bf),
            pltpu.VMEM((D, F), bf),
            pltpu.VMEM((F, D), bf),
            pltpu.VMEM((1, D), bf),
            pltpu.VMEM((D, 6 * D), bf),
            pltpu.VMEM((S, D), bf),
            pltpu.VMEM((S, D), jnp.float32),
            pltpu.VMEM((BQ, DH), bf),
            pltpu.VMEM((S, D), bf),
            pltpu.SemaphoreType.DMA(()),
            pltpu.SemaphoreType.DMA((len(WAIT_GROUPS),)),
            pltpu.SemaphoreType.DMA((RING,)),
            pltpu.SemaphoreType.DMA(()),
            pltpu.SemaphoreType.DMA(()),
        ],
        compiler_params=pltpu.CompilerParams(
            vmem_limit_bytes=100 * 1024 * 1024,
            flags={"XLA_TPU_RESCHEDULE_DMA_DONES": True},
        ),
    )(A_x.reshape(S, D), A_k_cache.reshape(H, SK, DH), A_v_cache.reshape(H, SK, DH),
      A_wq, A_wo, B_w_gate, B_w_up, B_w_down, c, w_mod)
    return out.reshape(1, S, D)
```
